```python
import os as _os
_os.environ.setdefault("JAX_PLATFORMS", "cpu")
import jax
import jax.numpy as jnp

def _softmax(x, axis=-1):
    return jax.nn.softmax(x, axis=axis)
def _gelu(x):
    return jax.nn.gelu(x, approximate=True)
def _silu(x):
    return jax.nn.silu(x)
def _sigmoid(x):
    return jax.nn.sigmoid(x)
def _layernorm(x, axis=-1, eps=1e-5):
    m = jnp.mean(x, axis=axis, keepdims=True)
    v = jnp.var(x, axis=axis, keepdims=True)
    return (x - m) / jnp.sqrt(v + eps)
def _scatter_add(tgt, idx, src, axis=0):
    return tgt.at[idx].add(src)
def _segment_sum(src, seg, n):
    return jax.ops.segment_sum(src, seg, n)
class _Rng:
    def __init__(self, key):
        self._k = key
    def _next(self):
        self._k, sub = jax.random.split(self._k)
        return sub
    def normal(self, shape):
        return jax.random.normal(self._next(), shape, dtype=jnp.bfloat16)
    def randint(self, lo, hi, shape):
        return jax.random.randint(self._next(), shape, lo, hi, dtype=jnp.int32)
    def uniform(self, shape, lo=0.0, hi=1.0):
        return jax.random.uniform(self._next(), shape, jnp.bfloat16, lo, hi)
    def permutation(self, n):
        return jax.random.permutation(self._next(), n)


kernel_name = 'concat_heads__gqa_block_cached__gqa_block_cached__near_ridge'

def setup_inputs():
    _rng = _Rng(jax.random.key(int.from_bytes(__import__("os").urandom(4), "little")))
    _w = (lambda a: (lambda t: t.astype(jnp.bfloat16) if jnp.issubdtype(t.dtype, jnp.floating) else t)(jnp.asarray(a)))
    def _A_setup():
        B, Sq, D = 16, 144, 448
        Hq, Hkv, Sk, Dh = 16, 8, 1024, 256
        assert Hq % Hkv == 0, (Hq, Hkv)
        return {
            "x": _w((lambda *s: _rng.normal(s) * 0.8)(B, Sq, D)),
            "k_cache": _w((lambda *s: _rng.normal(s) * 0.8)(B, Hkv, Sk, Dh)),
            "v_cache": _w((lambda *s: _rng.normal(s) * 0.05)(B, Hkv, Sk, Dh)),
            "wq": _w((lambda *s: _rng.normal(s) * 0.8)(D, Hq * Dh) * (D ** -0.5)),
            "wo": _w((lambda *s: _rng.normal(s) * 0.05)(Hq * Dh, D) * ((Hq * Dh) ** -0.5)),
        }
    _A_in = _A_setup()

    def _B_setup():
        B, Sq, D = 16, 144, 448
        Hq, Hkv, Sk, Dh = 16, 8, 1024, 256
        assert Hq % Hkv == 0, (Hq, Hkv)
        return {
            "x": _w((lambda *s: _rng.normal(s) * 0.8)(B, Sq, D)),
            "k_cache": _w((lambda *s: _rng.normal(s) * 0.8)(B, Hkv, Sk, Dh)),
            "v_cache": _w((lambda *s: _rng.normal(s) * 0.05)(B, Hkv, Sk, Dh)),
            "wq": _w((lambda *s: _rng.normal(s) * 0.8)(D, Hq * Dh) * (D ** -0.5)),
            "wo": _w((lambda *s: _rng.normal(s) * 0.05)(Hq * Dh, D) * ((Hq * Dh) ** -0.5)),
        }
    _B_in = _B_setup()

    return {
        "A_x": _A_in["x"],
        "A_k_cache": _A_in["k_cache"],
        "A_v_cache": _A_in["v_cache"],
        "A_wq": _A_in["wq"],
        "A_wo": _A_in["wo"],
        "B_x": _B_in["x"],
        "B_k_cache": _B_in["k_cache"],
        "B_v_cache": _B_in["v_cache"],
        "B_wq": _B_in["wq"],
        "B_wo": _B_in["wo"],
    }

def reference(A_x, A_k_cache, A_v_cache, A_wq, A_wo, B_x, B_k_cache, B_v_cache, B_wq, B_wo):
    def _A_ref(x, k_cache, v_cache, wq, wo):
        B, Sq, D = x.shape
        Hq, Dh = 16, 256
        Hkv = k_cache.shape[1]
        rep = Hq // Hkv
        q = (lambda x, *d: x.transpose(*d))((x @ wq).reshape(B, Sq, Hq, Dh), 0, 2, 1, 3)
        k = jnp.repeat(k_cache, rep, axis=1)
        v = jnp.repeat(v_cache, rep, axis=1)
        scores = jnp.einsum("bhqd,bhkd->bhqk", q, k) * (Dh ** -0.5)
        p = _softmax(scores, axis=-1)
        o = jnp.einsum("bhqk,bhkd->bhqd", p, v)
        return (lambda x, *d: x.transpose(*d))(o, 0, 2, 1, 3).reshape(B, Sq, Hq * Dh) @ wo

    def _B_ref(x, k_cache, v_cache, wq, wo):
        B, Sq, D = x.shape
        Hq, Dh = 16, 256
        Hkv = k_cache.shape[1]
        rep = Hq // Hkv
        q = (lambda x, *d: x.transpose(*d))((x @ wq).reshape(B, Sq, Hq, Dh), 0, 2, 1, 3)
        k = jnp.repeat(k_cache, rep, axis=1)
        v = jnp.repeat(v_cache, rep, axis=1)
        scores = jnp.einsum("bhqd,bhkd->bhqk", q, k) * (Dh ** -0.5)
        p = _softmax(scores, axis=-1)
        o = jnp.einsum("bhqk,bhkd->bhqd", p, v)
        return (lambda x, *d: x.transpose(*d))(o, 0, 2, 1, 3).reshape(B, Sq, Hq * Dh) @ wo

    a = _A_ref(A_x, A_k_cache, A_v_cache, A_wq, A_wo)
    b = _B_ref(B_x, B_k_cache, B_v_cache, B_wq, B_wo)
    return jnp.concatenate([a, b], axis=-1)
```

```python
import functools
import jax, jax.numpy as jnp
from jax import lax
import jax.experimental.pallas as pl
import jax.experimental.pallas.tpu as pltpu

B, Sq, D, Hq, Hkv, Sk, Dh = 16, 144, 448, 16, 8, 1024, 256
LOG2E = 1.4426950408889634
NT = (((1,), (1,)), ((), ()))
f32, bf16 = jnp.float32, jnp.bfloat16

def run(A_x, A_k, A_v, A_wq, A_wo, B_x, B_k, B_v, B_wq, B_wo, nbr=2, split=6, flags=None, nobc=True, qh=1, lag=None, pscr=False, sscr=False):
    nb = 8
    G = B // nb
    T = nb * Sq
    NIT = G * Hkv * (2 // nbr)
    NQ = 2 * Hkv // qh
    W = 2 * Dh
    c = LOG2E * Dh ** -0.5

    def body(xa, ka, va, wqa, woa, xb, kb, vb, wqb, wob, out, xbuf, kbuf, vbuf, wqbuf, wobuf, q_scr, o_scr, acc, stage,
             sem_x, sem_k, sem_v, sem_wq, sem_wo, sem_o):
        xs, ks, vs, wqs, wos = (xa, xb), (ka, kb), (va, vb), (wqa, wqb), (woa, wob)

        def x_copy(br): return pltpu.make_async_copy(xs[br], xbuf.at[br], sem_x.at[br])
        def wq_copy(br, j, slot):
            return pltpu.make_async_copy(wqs[br].at[:, pl.ds(j * qh * W, qh * W)], wqbuf.at[slot], sem_wq.at[slot])
        def kv_copies(br, g, h, slot, i):
            return [pltpu.make_async_copy(ks[br].at[pl.ds(g * nb, nb), h], kbuf.at[slot, i], sem_k.at[slot, i]),
                    pltpu.make_async_copy(vs[br].at[pl.ds(g * nb, nb), h], vbuf.at[slot, i], sem_v.at[slot, i]),
                    pltpu.make_async_copy(wos[br].at[:, pl.ds(h * W, W)], wobuf.at[slot, i], sem_wo.at[slot, i])]

        def wq_piece(br, h0, h1, s):
            return pltpu.make_async_copy(wqs[br].at[:, h0 * W:h1 * W], wqbuf.at[br, :, h0 * W:h1 * W], sem_wq.at[s])
        pieces = [wq_piece(0, 0, qh, 0), wq_piece(0, qh, 2 * qh, 1), wq_piece(0, 2 * qh, Hkv, 2), wq_piece(1, 0, Hkv, 3)]
        x_copy(0).start(); pieces[0].start()
        acc[...] = jnp.zeros(acc.shape, f32)
        x_copy(0).wait(); pieces[0].wait()
        pieces[1].start()
        H = NQ // 2

        def qstep(it, carry):
            br, j = it // H, it % H
            @pl.when(it == 1)
            def _():
                pieces[1].wait(); pieces[2].start()
            @pl.when(it == 2)
            def _():
                pieces[2].wait(); pieces[3].start(); x_copy(1).start()
            @pl.when(it == H)
            def _():
                pieces[3].wait(); x_copy(1).wait()
                for i in range(nbr):
                    for cp in kv_copies(i, 0, 0, 0, i): cp.start()
            x = xbuf[br]
            for t in range(qh):
                col = pl.multiple_of((j * qh + t) * W, W)
                q = jnp.dot(x, wqbuf[br, :, pl.ds(col, W)], preferred_element_type=f32).astype(bf16)
                q_scr[br, j * qh + t] = q
            return carry
        lax.fori_loop(0, NQ, qstep, 0)

        def decode(it):
            if nbr == 2: return 0, it // Hkv, it % Hkv
            return it % 2, it // (2 * Hkv), (it // 2) % Hkv

        def step(it, carry):
            br0, g, h = decode(it)
            slot = it % 2
            nb0, ng, nh = decode(it + 1)
            if nbr == 2:
                @pl.when(it + 1 < NIT)
                def _():
                    for i in range(2):
                        for cp in kv_copies(i, ng, nh, 1 - slot, i): cp.start()
            else:
                @pl.when(jnp.logical_and(it + 1 < NIT, nb0 == 0))
                def _():
                    for cp in kv_copies(0, ng, nh, 1 - slot, 0): cp.start()
                @pl.when(nb0 == 1)
                def _():
                    for cp in kv_copies(1, ng, nh, 1 - slot, 0): cp.start()
            for i in range(nbr):
                for cp in kv_copies(i, g, h, slot, i): cp.wait()
            t0 = pl.multiple_of(g * T, T)

            def qk(i, u):
                br = i if nbr == 2 else br0
                rows = pl.ds(t0 + u * Sq, Sq)
                q2 = jnp.concatenate([q_scr[br, h, rows, :Dh], q_scr[br, h, rows, Dh:]], axis=0)
                return lax.dot_general(q2, kbuf[slot, i, u], NT, preferred_element_type=f32)

            def pv(i, u, s):
                m = jnp.max(s, axis=-1, keepdims=True)
                p = jnp.exp2((s - m) * c)
                l = jnp.sum(p, axis=-1, keepdims=True)
                o = jnp.dot(p.astype(bf16), vbuf[slot, i, u], preferred_element_type=f32)
                o = (o * (1.0 / l)).astype(bf16)
                o_scr[i, u * Sq:(u + 1) * Sq, :Dh] = o[:Sq]
                o_scr[i, u * Sq:(u + 1) * Sq, Dh:] = o[Sq:]

            def oproj(i, n0, n1):
                if n0 == n1: return
                r = lax.dot_general(wobuf[slot, i], o_scr[i, n0 * 128:n1 * 128, :], NT, preferred_element_type=f32)
                row = i * D if nbr == 2 else pl.multiple_of(br0 * D, 64)
                acc[pl.ds(row, D), n0 * 128:n1 * 128] += r

            units = [(i, u) for i in range(nbr) for u in range(nb)]
            if lag is None:
                s = qk(*units[0])
                for n, (i, u) in enumerate(units):
                    if n + 1 < len(units):
                        s_next = qk(*units[n + 1])
                    else:
                        for i2 in range(nbr - 1): oproj(i2, 0, 9)
                        oproj(i, 0, split)
                    pv(i, u, s)
                    s = s_next
                oproj(nbr - 1, split, 9)
            else:
                todo = [(i, t, i * nb + min(t, nb - 1)) for i in range(nbr) for t in range(9)]
                s = qk(*units[0])
                for n, (i, u) in enumerate(units):
                    if n + 1 < len(units):
                        s_next = qk(*units[n + 1])
                    while todo and todo[0][2] <= n - lag:
                        i2, t, _ = todo.pop(0); oproj(i2, t, t + 1)
                    pv(i, u, s)
                    s = s_next
                for i2, t, _ in todo: oproj(i2, t, t + 1)

            last = (h == Hkv - 1) if nbr == 2 else jnp.logical_and(h == Hkv - 1, br0 == 1)
            @pl.when(last)
            def _():
                @pl.when(g > 0)
                def _():
                    pltpu.make_async_copy(stage, out.at[pl.ds((g - 1) * T, T)], sem_o).wait()
                stage[...] = acc[...].T.astype(bf16)
                acc[...] = jnp.zeros(acc.shape, f32)
                pltpu.make_async_copy(stage, out.at[pl.ds(g * T, T)], sem_o).start()
            return carry

        lax.fori_loop(0, NIT, step, 0)
        pltpu.make_async_copy(stage, out.at[pl.ds((G - 1) * T, T)], sem_o).wait()

    hbm = pl.BlockSpec(memory_space=pltpu.HBM)
    res = pl.pallas_call(
        body,
        in_specs=[hbm] * 10, out_specs=hbm,
        out_shape=jax.ShapeDtypeStruct((B * Sq, 2 * D), bf16),
        scratch_shapes=[
            pltpu.VMEM((2, B * Sq, D), bf16), pltpu.VMEM((2, nbr, nb, Sk, Dh), bf16), pltpu.VMEM((2, nbr, nb, Sk, Dh), bf16),
            pltpu.VMEM((2, D, Hkv * W), bf16), pltpu.VMEM((2, nbr, D, W), bf16),
            pltpu.VMEM((2, Hkv, B * Sq, W), bf16), pltpu.VMEM((nbr, T, W), bf16),
            pltpu.VMEM((2 * D, T), f32), pltpu.VMEM((T, 2 * D), bf16),
            pltpu.SemaphoreType.DMA((2,)), pltpu.SemaphoreType.DMA((2, nbr)), pltpu.SemaphoreType.DMA((2, nbr)),
            pltpu.SemaphoreType.DMA((4,)), pltpu.SemaphoreType.DMA((2, nbr)), pltpu.SemaphoreType.DMA(()),
        ],
        compiler_params=pltpu.CompilerParams(vmem_limit_bytes=120 * 2**20, flags=flags, disable_bounds_checks=nobc),
    )(A_x.reshape(B * Sq, D), A_k, A_v, A_wq, A_wo.T, B_x.reshape(B * Sq, D), B_k, B_v, B_wq, B_wo.T)
    return res.reshape(B, Sq, 2 * D)


@jax.jit
def pallas_concat_heads__gqa_block_cached__gqa_block_cached__near_ridge_kernel(A_x, A_k_cache, A_v_cache, A_wq, A_wo, B_x, B_k_cache, B_v_cache, B_wq, B_wo):
    return run(A_x, A_k_cache, A_v_cache, A_wq, A_wo, B_x, B_k_cache, B_v_cache, B_wq, B_wo, nbr=2, lag=2, qh=2)
```

```python
import functools
import jax, jax.numpy as jnp
from jax import lax
import jax.experimental.pallas as pl
import jax.experimental.pallas.tpu as pltpu

B, Sq, D, Hq, Hkv, Sk, Dh = 16, 144, 448, 16, 8, 1024, 256
LOG2E = 1.4426950408889634
NT = (((1,), (1,)), ((), ()))
f32, bf16 = jnp.float32, jnp.bfloat16

def run(A_x, A_k, A_v, A_wq, A_wo, B_x, B_k, B_v, B_wq, B_wo, flags=None, qh=2, lag=2, nc=4, tail=(4, 4, 4, 4, 4, 4),
        dmapos=2, tb=False, og=1, chain=(), cl=1, qu=15, late=1, exact=False, pr=2 * Sq, early=3):
    nb = 8
    G = B // nb
    T = nb * Sq
    NTL = T // 128
    W = 2 * Dh
    C = Sk // nc
    c = LOG2E * Dh ** -0.5

    def body(xa, ka, va, wqa, woa, xb, kb, vb, wqb, wob, out, xbuf, kbuf, vbuf, wqbuf, wobuf, q_scr, o_scr, acc, stage,
             sem_p, sem_kv, sem_o):
        xs, ks, vs, wqs, wos = (xa, xb), (ka, kb), (va, vb), (wqa, wqb), (woa, wob)

        def x_piece(br, r0, r1, s):
            return pltpu.make_async_copy(xs[br].at[r0:r1], xbuf.at[br, r0:r1], sem_p.at[s])
        def wq_piece(br, h0, h1, s):
            return pltpu.make_async_copy(wqs[br].at[:, h0 * W:h1 * W], wqbuf.at[br, :, h0 * W:h1 * W], sem_p.at[s])
        def kv_copies(g, h, slot):
            cs = []
            for i in range(2):
                cs += [pltpu.make_async_copy(ks[i].at[pl.ds(g * nb, nb), h], kbuf.at[slot, i], sem_kv.at[slot, i, 0]),
                       pltpu.make_async_copy(vs[i].at[pl.ds(g * nb, nb), h], vbuf.at[slot, i], sem_kv.at[slot, i, 1]),
                       pltpu.make_async_copy(wos[i].at[:, pl.ds(h * W, W)], wobuf.at[slot, i], sem_kv.at[slot, i, 2])]
            return cs
        def out_copy(g, t0, t1):
            r0 = g * T + t0 * 128
            rows = pl.ds(r0 if isinstance(r0, int) else pl.multiple_of(r0, 128), (t1 - t0) * 128)
            return pltpu.make_async_copy(stage.at[rows], out.at[rows], sem_o.at[g, t0])
        ogroups = [(t, min(t + og, NTL)) for t in range(0, NTL, og)]

        def qproj(br, h, r0, nr):
            col = h * W if isinstance(h, int) else pl.multiple_of(h * W, W)
            rows = pl.ds(r0 if isinstance(r0, int) else pl.multiple_of(r0, nr), nr)
            q = jnp.dot(xbuf[br, rows], wqbuf[br, :, pl.ds(col, W)], preferred_element_type=f32)
            q_scr[br, h, rows] = (q * c).astype(bf16)

        R = B * Sq
        Q4 = T // 4
        st = [[x_piece(0, 0, Q4, 0), wq_piece(0, 0, 1, 1)],
              [x_piece(0, Q4, 3 * Q4, 2)],
              [x_piece(0, 3 * Q4, T, 3), wq_piece(0, 1, 2, 4)],
              [wq_piece(0, 2, 6, 5)],
              [x_piece(0, T, R, 6), wq_piece(0, 6, Hkv, 7), x_piece(1, 0, R, 8), wq_piece(1, 0, Hkv, 9)]]
        st.append(kv_copies(0, 0, 0))
        def send(k):
            for cp in st[k]: cp.start()
        def arrive(k):
            for cp in st[k]: cp.wait()
        for k in range(early): send(k)
        def clear(i, carry):
            acc[pl.ds(pl.multiple_of(i * 64, 64), 64), :] = jnp.zeros((64, T), f32)
            return carry
        lax.fori_loop(0, 2 * D // 64, clear, 0)
        arrive(0)
        if early <= 1: send(1)
        if early <= 2: send(2)
        qproj(0, 0, 0, Q4)
        arrive(1)
        if early <= 3: send(3)
        qproj(0, 0, Q4, 2 * Q4)
        arrive(2)
        qproj(0, 0, 3 * Q4, Q4)
        qproj(0, 1, 0, T)
        arrive(3)
        send(4)
        PP = T // pr
        NP = 2 * G * Hkv * PP

        def qstep(it, carry):
            @pl.when(it == 1)
            def _():
                arrive(4)
                send(5)
            for t in range(qu):
                j = 2 * PP + it * qu + t
                qproj(j // (G * Hkv * PP), (j // PP) % Hkv, ((j // (Hkv * PP)) % G) * T + (j % PP) * pr, pr)
            return carry
        assert (NP - 2 * PP) % qu == 0 and 2 * PP + qu <= 6 * PP
        lax.fori_loop(0, (NP - 2 * PP) // qu, qstep, 0)

        def lane_tiles(a):
            return [a[:, j * 128:(j + 1) * 128] for j in range(a.shape[1] // 128)]

        def step(it, carry):
            g, h = it // Hkv, it % Hkv
            slot = it % 2
            def prefetch():
                @pl.when(it + 1 < G * Hkv)
                def _():
                    for cp in kv_copies((it + 1) // Hkv, (it + 1) % Hkv, 1 - slot): cp.start()
            if dmapos is None: prefetch()
            for cp in kv_copies(g, h, slot): cp.wait()
            t0 = pl.multiple_of(g * T, T)

            def load_q(i, u):
                rows = pl.ds(t0 + u * Sq, Sq)
                return jnp.concatenate([q_scr[i, h, rows, :Dh], q_scr[i, h, rows, Dh:]], axis=0)

            def qk(i, u, q2, k):
                return lax.dot_general(q2, kbuf[slot, i, u, k * C:(k + 1) * C, :], NT, preferred_element_type=f32)

            def rowmax(ss):
                t = functools.reduce(jnp.maximum, [x for s_ in ss for x in lane_tiles(s_)])
                return jnp.max(t, axis=-1, keepdims=True)

            def put_o(i, u, o, lp):
                l = jnp.sum(lp, axis=-1, keepdims=True)
                if exact: r = 1.0 / l
                else:
                    r = pl.reciprocal(l, approx=True)
                    r = r * (2.0 - l * r)
                o = (o * r).astype(bf16)
                o_scr[i, u * Sq:(u + 1) * Sq, :Dh] = o[:Sq]
                o_scr[i, u * Sq:(u + 1) * Sq, Dh:] = o[Sq:]

            def oproj(i, t):
                cols = slice(t * 128, (t + 1) * 128)
                r = lax.dot_general(wobuf[slot, i], o_scr[i, cols, :], NT, preferred_element_type=f32)
                prev = acc[i * D:(i + 1) * D, cols]
                r = jnp.where(h > 0, prev, 0.0) + r
                acc[i * D:(i + 1) * D, cols] = r
                if i == 1 and t < NTL - late: finish(t, jnp.concatenate([acc[:D, cols], r], axis=0))

            def finish(t, full, g=g, send=h == Hkv - 1):
                stage[pl.ds(pl.multiple_of(g * T, T) + t * 128, 128), :] = full.astype(bf16).T if tb else full.T.astype(bf16)
                for a, b_ in ogroups:
                    if b_ == t + 1:
                        @pl.when(send)
                        def _(): out_copy(g, a, b_).start()

            units = [(i, u) for i in range(2) for u in range(nb)]
            N = len(units)
            pos = [min((t // NTL) * nb + min(t % NTL, nb - 1) + lag, N) * nc for t in range(2 * NTL)]
            if tail is not None:
                for j, p_ in enumerate(tail): pos[2 * NTL - len(tail) + j] = (N - 1) * nc + p_
                for t in range(2 * NTL - 2, -1, -1): pos[t] = min(pos[t], pos[t + 1])
            todo = [(t // NTL, t % NTL, pos[t]) for t in range(2 * NTL)]
            q2 = load_q(*units[0])
            cur = [qk(*units[0], q2, k) for k in range(nc)]
            for n, (i, u) in enumerate(units):
                more = n + 1 < N
                if more: q2 = load_q(*units[n + 1])
                if dmapos == n: prefetch()
                nxt = []
                m = jnp.broadcast_to(rowmax(cur), (2 * Sq, 128))
                o = lp = None
                lps = []
                for k in range(nc):
                    if more: nxt.append(qk(*units[n + 1], q2, k))
                    while todo and todo[0][2] <= n * nc + k:
                        i2, a, _ = todo.pop(0); oproj(i2, a)
                    ps = [jnp.exp2(x - m) for x in lane_tiles(cur[k])]
                    for p in ps: lp = p if lp is None else lp + p
                    lps.append(lp)
                    if n in chain and k + 1 >= cl: m = jnp.where(lps[k + 1 - cl] < 0.0, lps[k + 1 - cl], m)
                    p = jnp.concatenate(ps, axis=1).astype(bf16)
                    d = jnp.dot(p, vbuf[slot, i, u, k * C:(k + 1) * C, :], preferred_element_type=f32)
                    o = d if o is None else o + d
                put_o(i, u, o, lp)
                cur = nxt
            for i2, a, _ in todo: oproj(i2, a)

            if late:
                @pl.when(h == Hkv - 1)
                def _():
                    for t in range(NTL - late, NTL): finish(t, acc[:, t * 128:(t + 1) * 128])
            return carry
        lax.fori_loop(0, G * Hkv, step, 0)
        for g in range(G):
            for a, b_ in ogroups: out_copy(g, a, b_).wait()

    hbm = pl.BlockSpec(memory_space=pltpu.HBM)
    res = pl.pallas_call(
        body,
        in_specs=[hbm] * 10, out_specs=hbm,
        out_shape=jax.ShapeDtypeStruct((B * Sq, 2 * D), bf16),
        scratch_shapes=[
            pltpu.VMEM((2, B * Sq, D), bf16), pltpu.VMEM((2, 2, nb, Sk, Dh), bf16), pltpu.VMEM((2, 2, nb, Sk, Dh), bf16),
            pltpu.VMEM((2, D, Hkv * W), bf16), pltpu.VMEM((2, 2, D, W), bf16),
            pltpu.VMEM((2, Hkv, B * Sq, W), bf16), pltpu.VMEM((2, T, W), bf16),
            pltpu.VMEM((2 * D, T), f32), pltpu.VMEM((B * Sq, 2 * D), bf16),
            pltpu.SemaphoreType.DMA((10,)), pltpu.SemaphoreType.DMA((2, 2, 3)), pltpu.SemaphoreType.DMA((G, NTL)),
        ],
        compiler_params=pltpu.CompilerParams(vmem_limit_bytes=124 * 2**20, flags=flags, disable_bounds_checks=True),
    )(A_x.reshape(B * Sq, D), A_k, A_v, A_wq, A_wo.T, B_x.reshape(B * Sq, D), B_k, B_v, B_wq, B_wo.T)
    return res.reshape(B, Sq, 2 * D)


@jax.jit
def pallas_concat_heads__gqa_block_cached__gqa_block_cached__near_ridge_kernel(A_x, A_k_cache, A_v_cache, A_wq, A_wo, B_x, B_k_cache, B_v_cache, B_wq, B_wo):
    return run(A_x, A_k_cache, A_v_cache, A_wq, A_wo, B_x, B_k_cache, B_v_cache, B_wq, B_wo, )
```

```python
import functools

import jax
import jax.numpy as jnp
from jax import lax
import jax.experimental.pallas as pl
import jax.experimental.pallas.tpu as pltpu

B, SQ, D = 16, 144, 448
HKV, SK, DH = 8, 1024, 256
W = 2 * DH
NB = 8
G = B // NB
T = NB * SQ
LANES = 128
NTILE = T // LANES
NCHUNK = 4
CHUNK = SK // NCHUNK
PIECE = T // 4
PIECES_PER_STEP = 15
A_COLS = D // LANES * LANES
Q_SCALE = 1.4426950408889634 * DH ** -0.5

F32, BF16 = jnp.float32, jnp.bfloat16
NT_DIMS = (((1,), (1,)), ((), ()))


def _div(a, n):
    return lax.shift_right_logical(a, n.bit_length() - 1)


def _mod(a, n):
    return a & (n - 1)


def _aligned(i, n):
    return i if isinstance(i, int) else pl.multiple_of(i, n)


def _lane_tiles(a):
    return [a[:, j:j + LANES] for j in range(0, a.shape[1], LANES)]


def _kernel(xa, ka, va, wqa, woa, xb, kb, vb, wqb, wob, out,
            x_buf, wq_buf, kv_buf, wo_buf, qa_buf, qb_buf, o_buf, acc, stage,
            sem_in, sem_kv, sem_wo, sem_out):
    xs, ks, vs, wqs, wos = (xa, xb), (ka, kb), (va, vb), (wqa, wqb), (woa, wob)

    def x_copy(br, r0, r1, s):
        return pltpu.make_async_copy(xs[br].at[r0:r1], x_buf.at[br, r0:r1], sem_in.at[s])

    def wq_copy(br, h0, h1, s):
        return pltpu.make_async_copy(wqs[br].at[:, h0 * W:h1 * W],
                                     wq_buf.at[br, :, h0 * W:h1 * W], sem_in.at[s])

    def kv_copies(g, h, slot):
        copies = []
        for br in range(2):
            copies += [
                pltpu.make_async_copy(ks[br].at[pl.ds(g * NB, NB), h],
                                      kv_buf.at[slot, br, 0], sem_kv.at[slot]),
                pltpu.make_async_copy(vs[br].at[pl.ds(g * NB, NB), h],
                                      kv_buf.at[slot, br, 1], sem_kv.at[slot]),
                pltpu.make_async_copy(wos[br].at[:, pl.ds(h * W, W)],
                                      wo_buf.at[slot, br], sem_wo.at[slot]),
            ]
        return copies

    def kv_wait(slot):
        pltpu.make_async_copy(kv_buf.at[slot], kv_buf.at[slot], sem_kv.at[slot]).wait()
        pltpu.make_async_copy(wo_buf.at[slot], wo_buf.at[slot], sem_wo.at[slot]).wait()

    def out_copy(g, t):
        rows = pl.ds(_aligned(g * T + t * LANES, LANES), LANES)
        return pltpu.make_async_copy(stage.at[rows], out.at[rows], sem_out.at[g, t])

    def q_proj(br, h, rows):
        q = jnp.dot(x_buf[br, rows], wq_buf[br, :, pl.ds(_aligned(h * W, W), W)],
                    preferred_element_type=F32)
        return (q * Q_SCALE).astype(BF16)

    def q_proj_a(h, r0, n):
        rows = pl.ds(_aligned(r0, n), n)
        qa_buf[h, rows] = q_proj(0, h, rows)

    stages = [
        [x_copy(0, 0, PIECE, 0), wq_copy(0, 0, 1, 1)],
        [x_copy(0, PIECE, 3 * PIECE, 2)],
        [x_copy(0, 3 * PIECE, T, 3)],
        [wq_copy(0, 1, 5, 4)],
        [x_copy(0, T, G * T, 5), wq_copy(0, 5, HKV, 6)],
        [x_copy(1, 0, G * T, 7), wq_copy(1, 0, HKV, 8)],
    ]

    def send(copies):
        for copy in copies:
            copy.start()

    def arrive(copies):
        for copy in copies:
            copy.wait()

    for copies in stages[:4]:
        send(copies)

    def clear(i, carry):
        acc[pl.ds(pl.multiple_of(i * 64, 64), 64), :] = jnp.zeros((64, T), F32)
        return carry

    lax.fori_loop(0, 2 * D // 64, clear, 0)
    arrive(stages[0])
    q_proj_a(0, 0, PIECE)
    arrive(stages[1])
    q_proj_a(0, PIECE, 2 * PIECE)
    arrive(stages[2])
    q_proj_a(0, 3 * PIECE, PIECE)
    arrive(stages[3])
    send(stages[4])
    send(stages[5])

    per_head = T // PIECE
    left = G * HKV * per_head - per_head
    assert left % PIECES_PER_STEP == 0 and per_head + PIECES_PER_STEP <= 5 * per_head

    def q_step(it, carry):
        @pl.when(it == 0)
        def _():
            send(kv_copies(0, 0, 0))

        @pl.when(it == 1)
        def _():
            arrive(stages[4])

        for t in range(PIECES_PER_STEP):
            j = per_head + it * PIECES_PER_STEP + t
            q_proj_a(_mod(_div(j, per_head), HKV),
                     _div(j, HKV * per_head) * T + _mod(j, per_head) * PIECE, PIECE)
        return carry

    lax.fori_loop(0, left // PIECES_PER_STEP, q_step, 0)
    arrive(stages[5])

    units = [(br, u) for br in range(2) for u in range(NB)]
    last = len(units) - 1
    tiles = [(br, t, br * NB + min(t, NB - 1) + 2) for br in range(2) for t in range(NTILE)]
    tiles = tiles[:-6] + [(br, t, last + 1) for br, t, _ in tiles[-6:]]

    def step(it, carry):
        g, h, slot = _div(it, HKV), _mod(it, HKV), _mod(it, 2)
        kv_wait(slot)
        t0 = pl.multiple_of(g * T, T)

        def load_q(br, u):
            if br == 0:
                rows = pl.ds(t0 + u * SQ, SQ)
                heads = [qa_buf[h, rows, :DH], qa_buf[h, rows, DH:]]
            else:
                rows = slice(u * SQ, (u + 1) * SQ)
                heads = [qb_buf[rows, :DH], qb_buf[rows, DH:]]
            return jnp.concatenate(heads, axis=0)

        def scores(br, u, q, k):
            return lax.dot_general(q, kv_buf[slot, br, 0, u, k * CHUNK:(k + 1) * CHUNK, :],
                                   NT_DIMS, preferred_element_type=F32)

        def store_o(br, u, o, partial_sum):
            l = jnp.sum(partial_sum, axis=-1, keepdims=True)
            r = pl.reciprocal(l, approx=True)
            r = r * (2.0 - l * r)
            o = (o * r).astype(BF16)
            o_buf[br, u * SQ:(u + 1) * SQ, :DH] = o[:SQ]
            o_buf[br, u * SQ:(u + 1) * SQ, DH:] = o[SQ:]

        def stage_tile(t, c0, val):
            stage[pl.ds(t0 + t * LANES, LANES), c0:c0 + val.shape[0]] = val.astype(BF16).T

        def out_proj(br, t):
            cols = slice(t * LANES, (t + 1) * LANES)
            r = lax.dot_general(wo_buf[slot, br], o_buf[br, cols, :], NT_DIMS,
                                preferred_element_type=F32)
            r = jnp.where(h > 0, acc[br * D:(br + 1) * D, cols], 0.0) + r
            acc[br * D:(br + 1) * D, cols] = r
            if br == 0 and t == NTILE - 1:
                stage_tile(t, 0, r[:A_COLS])
            if br == 1 and t < NTILE - 1:
                stage_tile(t, 0, jnp.concatenate([acc[:D, cols], r], axis=0))

                @pl.when(h == HKV - 1)
                def _():
                    out_copy(g, t).start()

        todo = list(tiles)

        def project_tiles(n):
            while todo and todo[0][2] <= n:
                br, t, _ = todo.pop(0)
                out_proj(br, t)

        q = load_q(*units[0])
        cur = [scores(*units[0], q, k) for k in range(NCHUNK)]
        for n, (br, u) in enumerate(units):
            if n < last:
                q = load_q(*units[n + 1])
            if n == 0:
                @pl.when(it + 1 < G * HKV)
                def _():
                    send(kv_copies(_div(it + 1, HKV), _mod(it + 1, HKV), 1 - slot))

            m = functools.reduce(jnp.maximum, [x for s in cur for x in _lane_tiles(s)])
            m = jnp.broadcast_to(jnp.max(m, axis=-1, keepdims=True), (2 * SQ, LANES))
            nxt, o, partial_sum = [], None, None
            for k in range(NCHUNK):
                if n < last:
                    nxt.append(scores(*units[n + 1], q, k))
                project_tiles(n)
                if n < 2 and k == 2:
                    half = T // 2
                    qb_buf[n * half:(n + 1) * half] = q_proj(1, h, pl.ds(t0 + n * half, half))
                ps = [jnp.exp2(x - m) for x in _lane_tiles(cur[k])]
                for p in ps:
                    partial_sum = p if partial_sum is None else partial_sum + p
                pv = jnp.dot(jnp.concatenate(ps, axis=1).astype(BF16),
                             kv_buf[slot, br, 1, u, k * CHUNK:(k + 1) * CHUNK, :],
                             preferred_element_type=F32)
                o = pv if o is None else o + pv
            store_o(br, u, o, partial_sum)
            cur = nxt
        project_tiles(last + 1)

        @pl.when(h == HKV - 1)
        def _():
            t = NTILE - 1
            stage_tile(t, A_COLS, acc[A_COLS:, t * LANES:(t + 1) * LANES])
            out_copy(g, t).start()

        return carry

    lax.fori_loop(0, G * HKV, step, 0)
    for g in range(G):
        for t in range(NTILE):
            out_copy(g, t).wait()


@jax.jit
def pallas_concat_heads__gqa_block_cached__gqa_block_cached__near_ridge_kernel(
    A_x: jax.Array,
    A_k_cache: jax.Array,
    A_v_cache: jax.Array,
    A_wq: jax.Array,
    A_wo: jax.Array,
    B_x: jax.Array,
    B_k_cache: jax.Array,
    B_v_cache: jax.Array,
    B_wq: jax.Array,
    B_wo: jax.Array,
):
    hbm = pl.BlockSpec(memory_space=pltpu.HBM)
    out = pl.pallas_call(
        _kernel,
        in_specs=[hbm] * 10,
        out_specs=hbm,
        out_shape=jax.ShapeDtypeStruct((B * SQ, 2 * D), BF16),
        scratch_shapes=[
            pltpu.VMEM((2, B * SQ, D), BF16),
            pltpu.VMEM((2, D, HKV * W), BF16),
            pltpu.VMEM((2, 2, 2, NB, SK, DH), BF16),
            pltpu.VMEM((2, 2, D, W), BF16),
            pltpu.VMEM((HKV, B * SQ, W), BF16),
            pltpu.VMEM((T, W), BF16),
            pltpu.VMEM((2, T, W), BF16),
            pltpu.VMEM((2 * D, T), F32),
            pltpu.VMEM((B * SQ, 2 * D), BF16),
            pltpu.SemaphoreType.DMA((9,)),
            pltpu.SemaphoreType.DMA((2,)),
            pltpu.SemaphoreType.DMA((2,)),
            pltpu.SemaphoreType.DMA((G, NTILE)),
        ],
        compiler_params=pltpu.CompilerParams(
            vmem_limit_bytes=100 * 2**20,
            disable_bounds_checks=True,
        ),
    )(A_x.reshape(B * SQ, D), A_k_cache, A_v_cache, A_wq, A_wo.T,
      B_x.reshape(B * SQ, D), B_k_cache, B_v_cache, B_wq, B_wo.T)
    return out.reshape(B, SQ, 2 * D)
```

```python
import functools

import jax
import jax.numpy as jnp
from jax import lax
import jax.experimental.pallas as pl
import jax.experimental.pallas.tpu as pltpu

B, SQ, D = 16, 144, 448
HKV, SK, DH = 8, 1024, 256
W = 2 * DH
NB = 8
G = B // NB
T = NB * SQ
LANES = 128
NTILE = T // LANES
NCHUNK = 4
CHUNK = SK // NCHUNK
PIECE = T // 4
PIECES_PER_STEP = 15
A_COLS = D // LANES * LANES
Q_SCALE = 1.4426950408889634 * DH ** -0.5

F32, BF16 = jnp.float32, jnp.bfloat16
NT_DIMS = (((1,), (1,)), ((), ()))


def _div(a, n):
    return lax.shift_right_logical(a, n.bit_length() - 1)


def _mod(a, n):
    return a & (n - 1)


def _aligned(i, n):
    return i if isinstance(i, int) else pl.multiple_of(i, n)


def _lane_tiles(a):
    return [a[:, j:j + LANES] for j in range(0, a.shape[1], LANES)]


def _kernel(xa, ka, va, wqa, woa, xb, kb, vb, wqb, wob, out,
            x_buf, wq_buf, kv_buf, wo_buf, qa_buf, qb_buf, o_buf, acc, stage,
            sem_in, sem_kv, sem_wo, sem_out):
    xs, ks, vs, wqs, wos = (xa, xb), (ka, kb), (va, vb), (wqa, wqb), (woa, wob)

    def x_copy(br, r0, r1, s):
        return pltpu.make_async_copy(xs[br].at[r0:r1], x_buf.at[br, r0:r1], sem_in.at[s])

    def wq_copy(br, h0, h1, s):
        return pltpu.make_async_copy(wqs[br].at[:, h0 * W:h1 * W],
                                     wq_buf.at[br, :, h0 * W:h1 * W], sem_in.at[s])

    def kv_copies(g, h, slot):
        copies = []
        for br in range(2):
            copies += [
                pltpu.make_async_copy(ks[br].at[pl.ds(g * NB, NB), h],
                                      kv_buf.at[slot, br, 0], sem_kv.at[slot]),
                pltpu.make_async_copy(vs[br].at[pl.ds(g * NB, NB), h],
                                      kv_buf.at[slot, br, 1], sem_kv.at[slot]),
                pltpu.make_async_copy(wos[br].at[:, pl.ds(h * W, W)],
                                      wo_buf.at[slot, br], sem_wo.at[slot]),
            ]
        return copies

    def kv_wait(slot):
        pltpu.make_async_copy(kv_buf.at[slot], kv_buf.at[slot], sem_kv.at[slot]).wait()
        pltpu.make_async_copy(wo_buf.at[slot], wo_buf.at[slot], sem_wo.at[slot]).wait()

    def out_copy(g, t):
        rows = pl.ds(_aligned(g * T + t * LANES, LANES), LANES)
        return pltpu.make_async_copy(stage.at[rows], out.at[rows], sem_out.at[g, t])

    def q_proj(br, h, rows):
        q = jnp.dot(x_buf[br, rows], wq_buf[br, :, pl.ds(_aligned(h * W, W), W)],
                    preferred_element_type=F32)
        return (q * Q_SCALE).astype(BF16)

    def q_proj_a(h, r0, n):
        rows = pl.ds(_aligned(r0, n), n)
        qa_buf[h, rows] = q_proj(0, h, rows)

    stages = [
        [x_copy(0, 0, PIECE, 0), wq_copy(0, 0, 1, 1)],
        [x_copy(0, PIECE, 3 * PIECE, 2)],
        [x_copy(0, 3 * PIECE, T, 3)],
        [wq_copy(0, 1, 5, 4)],
        [x_copy(0, T, G * T, 5), wq_copy(0, 5, HKV, 6)],
        [x_copy(1, 0, G * T, 7), wq_copy(1, 0, HKV, 8)],
    ]

    def send(copies):
        for copy in copies:
            copy.start()

    def arrive(copies):
        for copy in copies:
            copy.wait()

    for copies in stages[:4]:
        send(copies)

    def clear(i, carry):
        acc[pl.ds(pl.multiple_of(i * 64, 64), 64), :] = jnp.zeros((64, T), F32)
        return carry

    lax.fori_loop(0, 2 * D // 64, clear, 0)
    arrive(stages[0])
    q_proj_a(0, 0, PIECE)
    arrive(stages[1])
    q_proj_a(0, PIECE, 2 * PIECE)
    arrive(stages[2])
    q_proj_a(0, 3 * PIECE, PIECE)
    arrive(stages[3])
    send(stages[4])
    send(stages[5])

    per_head = T // PIECE
    left = G * HKV * per_head - per_head
    assert left % PIECES_PER_STEP == 0 and per_head + PIECES_PER_STEP <= 5 * per_head

    def q_step(it, carry):
        @pl.when(it == 0)
        def _():
            send(kv_copies(0, 0, 0))

        @pl.when(it == 1)
        def _():
            arrive(stages[4])

        for t in range(PIECES_PER_STEP):
            j = per_head + it * PIECES_PER_STEP + t
            q_proj_a(_mod(_div(j, per_head), HKV),
                     _div(j, HKV * per_head) * T + _mod(j, per_head) * PIECE, PIECE)
        return carry

    lax.fori_loop(0, left // PIECES_PER_STEP, q_step, 0)
    arrive(stages[5])

    units = [(br, u) for br in range(2) for u in range(NB)]
    last = len(units) - 1
    tiles = [(br, t, (br * NB + min(t, NB - 1) + 2, 0)) for br in range(2) for t in range(NTILE)]
    tail = 2 * [(last, NCHUNK - 1)] + 4 * [(last + 1, 0)]
    tiles[-len(tail):] = [(br, t, at) for (br, t, _), at in zip(tiles[-len(tail):], tail)]

    def step(it, carry):
        g, h, slot = _div(it, HKV), _mod(it, HKV), _mod(it, 2)
        kv_wait(slot)
        t0 = pl.multiple_of(g * T, T)

        def load_q(br, u):
            if br == 0:
                rows = pl.ds(t0 + u * SQ, SQ)
                heads = [qa_buf[h, rows, :DH], qa_buf[h, rows, DH:]]
            else:
                rows = slice(u * SQ, (u + 1) * SQ)
                heads = [qb_buf[rows, :DH], qb_buf[rows, DH:]]
            return jnp.concatenate(heads, axis=0)

        def scores(br, u, q, k):
            return lax.dot_general(q, kv_buf[slot, br, 0, u, k * CHUNK:(k + 1) * CHUNK, :],
                                   NT_DIMS, preferred_element_type=F32)

        def store_o(br, u, o, partial_sum):
            l = jnp.sum(partial_sum, axis=-1, keepdims=True)
            r = pl.reciprocal(l, approx=True)
            r = r * (2.0 - l * r)
            o = (o * r).astype(BF16)
            o_buf[br, u * SQ:(u + 1) * SQ, :DH] = o[:SQ]
            o_buf[br, u * SQ:(u + 1) * SQ, DH:] = o[SQ:]

        def stage_tile(t, c0, val):
            stage[pl.ds(t0 + t * LANES, LANES), c0:c0 + val.shape[0]] = val.astype(BF16).T

        def out_proj(br, t):
            cols = slice(t * LANES, (t + 1) * LANES)
            r = lax.dot_general(wo_buf[slot, br], o_buf[br, cols, :], NT_DIMS,
                                preferred_element_type=F32)
            r = jnp.where(h > 0, acc[br * D:(br + 1) * D, cols], 0.0) + r
            acc[br * D:(br + 1) * D, cols] = r
            if br == 0 and t == NTILE - 1:
                stage_tile(t, 0, r[:A_COLS])
            if br == 1 and t < NTILE - 1:
                stage_tile(t, 0, jnp.concatenate([acc[:D, cols], r], axis=0))

                @pl.when(h == HKV - 1)
                def _():
                    out_copy(g, t).start()

        todo = list(tiles)

        def project_tiles(n, k):
            while todo and todo[0][2] <= (n, k):
                br, t, _ = todo.pop(0)
                out_proj(br, t)

        q = load_q(*units[0])
        cur = [scores(*units[0], q, k) for k in range(NCHUNK)]
        for n, (br, u) in enumerate(units):
            if n < last:
                q = load_q(*units[n + 1])
            if n == 0:
                @pl.when(it + 1 < G * HKV)
                def _():
                    send(kv_copies(_div(it + 1, HKV), _mod(it + 1, HKV), 1 - slot))

            m = functools.reduce(jnp.maximum, [x for s in cur for x in _lane_tiles(s)])
            m = jnp.broadcast_to(jnp.max(m, axis=-1, keepdims=True), (2 * SQ, LANES))
            nxt, o, partial_sum = [], None, None
            for k in range(NCHUNK):
                if n < last:
                    nxt.append(scores(*units[n + 1], q, k))
                project_tiles(n, k)
                if n < 2 and k == 2:
                    half = T // 2
                    qb_buf[n * half:(n + 1) * half] = q_proj(1, h, pl.ds(t0 + n * half, half))
                ps = [jnp.exp2(x - m) for x in _lane_tiles(cur[k])]
                for p in ps:
                    partial_sum = p if partial_sum is None else partial_sum + p
                pv = jnp.dot(jnp.concatenate(ps, axis=1).astype(BF16),
                             kv_buf[slot, br, 1, u, k * CHUNK:(k + 1) * CHUNK, :],
                             preferred_element_type=F32)
                o = pv if o is None else o + pv
            store_o(br, u, o, partial_sum)
            cur = nxt
        project_tiles(last + 1, 0)

        @pl.when(h == HKV - 1)
        def _():
            t = NTILE - 1
            stage_tile(t, A_COLS, acc[A_COLS:, t * LANES:(t + 1) * LANES])
            out_copy(g, t).start()

        return carry

    lax.fori_loop(0, G * HKV, step, 0)
    for g in range(G):
        for t in range(NTILE):
            out_copy(g, t).wait()


@jax.jit
def pallas_concat_heads__gqa_block_cached__gqa_block_cached__near_ridge_kernel(
    A_x: jax.Array,
    A_k_cache: jax.Array,
    A_v_cache: jax.Array,
    A_wq: jax.Array,
    A_wo: jax.Array,
    B_x: jax.Array,
    B_k_cache: jax.Array,
    B_v_cache: jax.Array,
    B_wq: jax.Array,
    B_wo: jax.Array,
):
    hbm = pl.BlockSpec(memory_space=pltpu.MemorySpace.HBM)
    out = pl.pallas_call(
        _kernel,
        in_specs=[hbm] * 10,
        out_specs=hbm,
        out_shape=jax.ShapeDtypeStruct((B * SQ, 2 * D), BF16),
        scratch_shapes=[
            pltpu.VMEM((2, B * SQ, D), BF16),
            pltpu.VMEM((2, D, HKV * W), BF16),
            pltpu.VMEM((2, 2, 2, NB, SK, DH), BF16),
            pltpu.VMEM((2, 2, D, W), BF16),
            pltpu.VMEM((HKV, B * SQ, W), BF16),
            pltpu.VMEM((T, W), BF16),
            pltpu.VMEM((2, T, W), BF16),
            pltpu.VMEM((2 * D, T), F32),
            pltpu.VMEM((B * SQ, 2 * D), BF16),
            pltpu.SemaphoreType.DMA((9,)),
            pltpu.SemaphoreType.DMA((2,)),
            pltpu.SemaphoreType.DMA((2,)),
            pltpu.SemaphoreType.DMA((G, NTILE)),
        ],
        compiler_params=pltpu.CompilerParams(
            vmem_limit_bytes=100 * 2**20,
            disable_bounds_checks=True,
        ),
    )(A_x.reshape(B * SQ, D), A_k_cache, A_v_cache, A_wq, A_wo.T,
      B_x.reshape(B * SQ, D), B_k_cache, B_v_cache, B_wq, B_wo.T)
    return out.reshape(B, SQ, 2 * D)
```
